```python
import os as _os
_os.environ.setdefault("JAX_PLATFORMS", "cpu")
import jax
import jax.numpy as jnp

def _softmax(x, axis=-1):
    return jax.nn.softmax(x, axis=axis)
def _gelu(x):
    return jax.nn.gelu(x, approximate=True)
def _silu(x):
    return jax.nn.silu(x)
def _sigmoid(x):
    return jax.nn.sigmoid(x)
def _layernorm(x, axis=-1, eps=1e-5):
    m = jnp.mean(x, axis=axis, keepdims=True)
    v = jnp.var(x, axis=axis, keepdims=True)
    return (x - m) / jnp.sqrt(v + eps)
def _scatter_add(tgt, idx, src, axis=0):
    return tgt.at[idx].add(src)
def _segment_sum(src, seg, n):
    return jax.ops.segment_sum(src, seg, n)
class _Rng:
    def __init__(self, key):
        self._k = key
    def _next(self):
        self._k, sub = jax.random.split(self._k)
        return sub
    def normal(self, shape):
        return jax.random.normal(self._next(), shape, dtype=jnp.bfloat16)
    def randint(self, lo, hi, shape):
        return jax.random.randint(self._next(), shape, lo, hi, dtype=jnp.int32)
    def uniform(self, shape, lo=0.0, hi=1.0):
        return jax.random.uniform(self._next(), shape, jnp.bfloat16, lo, hi)
    def permutation(self, n):
        return jax.random.permutation(self._next(), n)


kernel_name = 'gated_mix__ssm_conv_s5__geglu_ffn__prompt'

def setup_inputs():
    _rng = _Rng(jax.random.key(int.from_bytes(__import__("os").urandom(4), "little")))
    _w = (lambda a: (lambda t: t.astype(jnp.bfloat16) if jnp.issubdtype(t.dtype, jnp.floating) else t)(jnp.asarray(a)))
    def _A_setup():
        B, S, D = 1, 2048, 512
        P = D
        Lambda_re = -0.5 * jnp.exp((lambda *s: _rng.normal(s) * 0.4)(P))
        Lambda_im = (lambda *s: _rng.normal(s) * 0.4)(P) * 1.0
        B_re = (lambda *s: _rng.normal(s) * 0.4)(P, D) * (D ** -0.5)
        B_im = (lambda *s: _rng.normal(s) * 0.4)(P, D) * (D ** -0.5)
        C_re = (lambda *s: _rng.normal(s) * 0.4)(D, P) * (P ** -0.5)
        C_im = (lambda *s: _rng.normal(s) * 0.4)(D, P) * (P ** -0.5)
        log_dt = (lambda *s: _rng.normal(s) * 0.4)(P) * 0.3 - 2.0
        Dskip = (lambda *s: _rng.normal(s) * 0.4)(D)
        return {
            "x": _w((lambda *s: _rng.normal(s) * 0.05)(B, S, D)),
            "Lambda_re": _w(Lambda_re),
            "Lambda_im": _w(Lambda_im),
            "B_re": _w(B_re),
            "B_im": _w(B_im),
            "C_re": _w(C_re),
            "C_im": _w(C_im),
            "log_dt": _w(log_dt),
            "Dskip": _w(Dskip),
        }
    _A_in = _A_setup()

    def _B_setup():
        B, S, D, F = 1, 2048, 512, 1376
        return {
            "x": _w((lambda *s: _rng.normal(s) * 0.05)(B, S, D)),
            "w_gate": _w((lambda *s: _rng.normal(s) * 0.1)(D, F)),
            "w_up": _w((lambda *s: _rng.normal(s) * 0.1)(D, F)),
            "w_down": _w((lambda *s: _rng.normal(s) * 0.1)(F, D)),
        }
    _B_in = _B_setup()

    return {
        "A_x": _A_in["x"],
        "A_Lambda_re": _A_in["Lambda_re"],
        "A_Lambda_im": _A_in["Lambda_im"],
        "A_B_re": _A_in["B_re"],
        "A_B_im": _A_in["B_im"],
        "A_C_re": _A_in["C_re"],
        "A_C_im": _A_in["C_im"],
        "A_log_dt": _A_in["log_dt"],
        "A_Dskip": _A_in["Dskip"],
        "B_x": _B_in["x"],
        "B_w_gate": _B_in["w_gate"],
        "B_w_up": _B_in["w_up"],
        "B_w_down": _B_in["w_down"],
        "gate_w": _w((lambda *s: _rng.normal(s) * 0.05)(512) * 16.0),
    }

def reference(A_x, A_Lambda_re, A_Lambda_im, A_B_re, A_B_im, A_C_re, A_C_im, A_log_dt, A_Dskip, B_x, B_w_gate, B_w_up, B_w_down, gate_w):
    def _A_ref(x, Lambda_re, Lambda_im, B_re, B_im, C_re, C_im, log_dt, Dskip):
        Bsz, L, H = x.shape
        Lam = Lambda_re + 1j * Lambda_im
        Bmat = B_re + 1j * B_im
        Cmat = C_re + 1j * C_im
        dt = jnp.exp(log_dt)
        Lam_bar = jnp.exp(dt * Lam)
        B_bar = ((Lam_bar - 1.0) / Lam)[:, None] * Bmat
        Bu = jnp.einsum("bld,pd->blp", x + 0j, B_bar)
        h = jnp.zeros_like(Bu[:, 0, :])
        hs = []
        for t in range(L):
            h = Lam_bar[None, :] * h + Bu[:, t, :]
            hs.append(h)
        hseq = jnp.stack(hs, 1)
        y = 2.0 * jnp.einsum("blp,dp->bld", hseq, Cmat).real + x * Dskip[None, None, :]
        return y

    def _B_ref(x, w_gate, w_up, w_down):
        return (_gelu(x @ w_gate) * (x @ w_up)) @ w_down

    x = A_x
    g = _sigmoid((x * gate_w).sum(-1, keepdims=True))
    a = _A_ref(x, A_Lambda_re, A_Lambda_im, A_B_re, A_B_im, A_C_re, A_C_im, A_log_dt, A_Dskip)
    b = _B_ref(x, B_w_gate, B_w_up, B_w_down)
    return g * a + (1 - g) * b
```

```python
import numpy as np
import jax
import jax.numpy as jnp
from jax import lax
import jax.experimental.pallas as pl
import jax.experimental.pallas.tpu as pltpu

T, D, P, F = 2048, 512, 512, 1376
TB = 512
FC = 256
OUT_BF16 = 0
UNROLL = 0
ORDER0 = "B0 W1 B1 B2 B3 W2 S0 S1 S2 S3 F0 F1 W3 F2 F3 F4 F5 W4 P G D0 C0 C1 C2 C3 O0 D1 O1 D2 O2 D3 O3".split()
ORDERN = "B0 S0 F0 B1 S1 F1 B2 S2 F2 B3 S3 F3 F4 F5 G C0 C1 C2 C3 D0 O0 D1 O1 D2 O2 D3 O3".split()
WGROUPS = [g.split(",") for g in "x0,b0 b1 f0 f1 c,d,xr".split()]
SCOPES = 0
NB = T // TB
LC = TB // 8
NT = (((1,), (1,)), ((), ()))
f32 = jnp.float32
bf16 = jnp.bfloat16
ODT = bf16 if OUT_BF16 else f32
C1 = float(np.sqrt(2.0 / np.pi))
C2 = float(np.sqrt(2.0 / np.pi) * 0.044715)
FCH = [(c0, min(c0 + FC, F)) for c0 in range(0, F, FC)]
NF = len(FCH)
FSPLIT = 512


class _null:
    def __enter__(self): pass
    def __exit__(self, *a): pass


def scope(n):
    return jax.named_scope(n) if SCOPES else _null()


def cmac(ar, ai, hr, hi, ur, ui):
    return ur + (ar * hr - ai * hi), ui + (ar * hi + ai * hr)


def _kernel(x_h, lre_h, lim_h, bre_h, bim_h, cre_h, cim_h, ldt_h, dsk_h, wg_h, wu_h, wd_h, gw_h, o_h,
            x_s, vec_s, b_s, c_s, ct_s, wg_s, wu_s, wd_s, act_s, tab_ref, h_ref, hb_s, us, ys, out_s,
            sems, osem):
    mk = pltpu.make_async_copy
    cp_vec = [mk(h, vec_s[n], sems.at[0]) for n, h in enumerate((lre_h, lim_h, ldt_h, dsk_h, gw_h))]
    cp_x = [mk(x_h.at[pl.ds(b * TB, TB)], x_s.at[b], sems.at[7 + b]) for b in range(NB)]
    cp_b0 = [mk((bre_h, bim_h)[k].at[0:128], b_s.at[k, 0:128], sems.at[1]) for k in range(2)]
    cp_b1 = [mk((bre_h, bim_h)[k].at[128:P], b_s.at[k, 128:P], sems.at[2]) for k in range(2)]
    cp_f0 = [mk(h.at[0:FSPLIT], s.at[0:FSPLIT], sems.at[3]) for h, s in ((wg_h, wg_s), (wu_h, wu_s))]
    cp_f1 = [mk(h.at[FSPLIT:F], s.at[FSPLIT:F], sems.at[4]) for h, s in ((wg_h, wg_s), (wu_h, wu_s))]
    cp_c = [mk((cre_h, cim_h)[k], c_s.at[k], sems.at[5]) for k in range(2)]
    cp_d = [mk(wd_h, wd_s, sems.at[6])]

    GR = dict(x0=cp_x[0:1], b0=cp_b0, b1=cp_b1, f0=cp_f0, f1=cp_f1, c=cp_c, d=cp_d, xr=cp_x[1:])
    WAITS = [[c for g in w for c in GR[g]] for w in WGROUPS]
    for grp in [cp_vec] + WAITS:
        for c in grp:
            c.start()

    with scope("prolog"):
        for c in cp_vec:
            c.wait()
        lre = vec_s[0][...].reshape(1, P).astype(f32)
        lim = vec_s[1][...].reshape(1, P).astype(f32)
        dt = jnp.exp(vec_s[2][...].reshape(1, P).astype(f32)).astype(bf16).astype(f32)
        zr = dt * lre
        zi = dt * lim
        a_m = jnp.exp(zr)
        ar = a_m * jnp.cos(zi)
        ai = a_m * jnp.sin(zi)
        s = lax.broadcasted_iota(jnp.int32, (8, P), 0)
        sf = ((s + 1) * LC).astype(f32)
        mg = jnp.exp(sf * zr)
        pr = mg * jnp.cos(sf * zi)
        pi = mg * jnp.sin(sf * zi)
        den = 1.0 / (lre * lre + lim * lim)
        nr = ar - 1.0
        cr2 = 2.0 * (nr * lre + ai * lim) * den
        ci2 = 2.0 * (ai * lre - nr * lim) * den
        tab_ref[0] = pr
        tab_ref[1] = pi
        for n, k in enumerate((1, 2, 4)):
            kr = jnp.broadcast_to(pr[k - 1:k, :], (8, P))
            ki = jnp.broadcast_to(pi[k - 1:k, :], (8, P))
            tab_ref[2 + 2 * n] = jnp.where(s >= k, kr, 0.0)
            tab_ref[3 + 2 * n] = jnp.where(s >= k, ki, 0.0)
        tab_ref[8] = jnp.broadcast_to(ar, (8, P))
        tab_ref[9] = jnp.broadcast_to(ai, (8, P))
        tab_ref[10] = jnp.broadcast_to(cr2, (8, P))
        tab_ref[11] = jnp.broadcast_to(ci2, (8, P))
        h_ref[...] = jnp.zeros(h_ref.shape, f32)

    def body(b, first):
        if first:
            with scope("w0"):
                for c in WAITS[0]:
                    c.wait()
        x = x_s[b]

        def bproj(q):
            sl = slice(128 * q, 128 * q + 128)
            for k in range(2):
                u = lax.dot_general(x, b_s[k, sl, :], NT, preferred_element_type=f32)
                for m in range(TB // 8):
                    c, jb = divmod(m, LC // 8)
                    us[2 * q + k, pl.ds(64 * jb + c, 8, stride=8), :] = u[8 * m:8 * m + 8, :]

        def scan(q):
            sl = slice(128 * q, 128 * q + 128)
            ar = tab_ref[8, :, sl]
            ai = tab_ref[9, :, sl]
            er = us[2 * q, 0:8, :]
            ei = us[2 * q + 1, 0:8, :]
            for j in range(1, LC):
                er, ei = cmac(ar, ai, er, ei, us[2 * q, 8 * j:8 * j + 8, :], us[2 * q + 1, 8 * j:8 * j + 8, :])
            for n, k in enumerate((1, 2, 4)):
                er, ei = cmac(tab_ref[2 + 2 * n, :, sl], tab_ref[3 + 2 * n, :, sl],
                              pltpu.roll(er, k, 0), pltpu.roll(ei, k, 0), er, ei)
            h0r = h_ref[0, :, sl]
            h0i = h_ref[1, :, sl]
            er, ei = cmac(tab_ref[0, :, sl], tab_ref[1, :, sl], h0r, h0i, er, ei)
            h_ref[0, :, sl] = jnp.broadcast_to(er[7:8, :], (8, 128))
            h_ref[1, :, sl] = jnp.broadcast_to(ei[7:8, :], (8, 128))
            sub = lax.broadcasted_iota(jnp.int32, (8, 128), 0)
            hr = jnp.where(sub == 0, h0r, pltpu.roll(er, 1, 0))
            hi = jnp.where(sub == 0, h0i, pltpu.roll(ei, 1, 0))
            for j in range(0, LC, 2):
                r0, i0 = cmac(ar, ai, hr, hi, us[2 * q, 8 * j:8 * j + 8, :], us[2 * q + 1, 8 * j:8 * j + 8, :])
                hr, hi = cmac(ar, ai, r0, i0, us[2 * q, 8 * j + 8:8 * j + 16, :], us[2 * q + 1, 8 * j + 8:8 * j + 16, :])
                hb_s[0, 8 * j:8 * j + 16, sl] = jnp.concatenate([r0, hr], axis=0).astype(bf16)
                hb_s[1, 8 * j:8 * j + 16, sl] = jnp.concatenate([i0, hi], axis=0).astype(bf16)

        def ffn(n):
            c0, c1 = FCH[n]
            g = lax.dot_general(x, wg_s[c0:c1, :], NT, preferred_element_type=f32)
            u = lax.dot_general(x, wu_s[c0:c1, :], NT, preferred_element_type=f32)
            z = g * (C1 + C2 * (g * g))
            gu = g * u
            act_s[:, c0:c1] = (gu + gu * jnp.tanh(z)).astype(bf16)

        def cprep():
            cr2 = tab_ref[10, 0:1, :]
            ci2 = tab_ref[11, 0:1, :]
            Cre = c_s[0].astype(f32)
            Cim = c_s[1].astype(f32)
            ct_s[0] = (Cre * cr2 - Cim * ci2).astype(bf16)
            ct_s[1] = (-(Cre * ci2 + Cim * cr2)).astype(bf16)

        def waitall(cps):
            for c in cps:
                c.wait()

        st = {}

        def gate():
            xf = x.astype(f32)
            gl = jnp.sum(xf * vec_s[4][...].reshape(1, D).astype(f32), axis=-1, keepdims=True)
            gt = jax.nn.sigmoid(gl)
            dsk = vec_s[3][...].reshape(1, D).astype(f32)
            st["xf"], st["gt"], st["dsk"] = xf, gt, dsk

        def cproj(n):
            sl = slice(128 * n, 128 * n + 128)
            y = lax.dot_general(hb_s[0], ct_s[0, sl, :], NT, preferred_element_type=f32)
            y = y + lax.dot_general(hb_s[1], ct_s[1, sl, :], NT, preferred_element_type=f32)
            ys[n] = y

        def dproj(n):
            sl = slice(128 * n, 128 * n + 128)
            st["acc", n] = jnp.dot(act_s[...], wd_s[:, sl], preferred_element_type=f32)

        def comb(n):
            sl = slice(128 * n, 128 * n + 128)
            parts = []
            for m in range(TB // 8):
                c, jb = divmod(m, LC // 8)
                parts.append(ys[n, pl.ds(64 * jb + c, 8, stride=8), :])
            gt = st["gt"]
            y = jnp.concatenate(parts, axis=0) + st["xf"][:, sl] * st["dsk"][:, sl]
            out_s[b, :, sl] = (gt * y + (0.5 - 0.5 * gt) * st["acc", n]).astype(ODT)
            mk(out_s.at[b, :, sl], o_h.at[pl.ds(b * TB, TB), sl], osem.at[0]).start()

        for tok in (ORDER0 if first else ORDERN):
            k, n = tok[0], int(tok[1:]) if len(tok) > 1 else 0
            if k == "W":
                with scope("w%d" % n):
                    waitall(WAITS[n])
            elif k == "B": bproj(n)
            elif k == "S": scan(n)
            elif k == "F": ffn(n)
            elif k == "P": cprep()
            elif k == "G": gate()
            elif k == "C": cproj(n)
            elif k == "D": dproj(n)
            elif k == "O": comb(n)

    with scope("body0"):
        body(0, True)

    def loop(b, carry):
        with scope("bodyN"):
            body(b, False)
        return carry

    if UNROLL:
        for b in range(1, NB):
            with scope("bodyN"):
                body(b, False)
    else:
        lax.fori_loop(1, NB, loop, 0)
    with scope("tail"):
        mk(out_s, out_s, osem.at[0]).wait()


@jax.jit
def pallas_gated_mix__ssm_conv_s5__geglu_ffn__prompt_kernel(
    A_x, A_Lambda_re, A_Lambda_im, A_B_re, A_B_im, A_C_re, A_C_im, A_log_dt, A_Dskip,
    B_x, B_w_gate, B_w_up, B_w_down, gate_w,
):
    x = A_x.reshape(T, D)
    hbm = pl.BlockSpec(memory_space=pltpu.HBM)
    out = pl.pallas_call(
        _kernel,
        in_specs=[hbm] * 13,
        out_specs=hbm,
        out_shape=jax.ShapeDtypeStruct((T, D), ODT),
        scratch_shapes=[
            pltpu.VMEM((NB, TB, D), bf16),
            [pltpu.VMEM((512,), bf16)] * 5,
            pltpu.VMEM((2, P, D), bf16),
            pltpu.VMEM((2, D, P), bf16),
            pltpu.VMEM((2, D, P), bf16),
            pltpu.VMEM((F, D), bf16),
            pltpu.VMEM((F, D), bf16),
            pltpu.VMEM((F, D), bf16),
            pltpu.VMEM((TB, F), bf16),
            pltpu.VMEM((12, 8, P), f32),
            pltpu.VMEM((2, 8, P), f32),
            pltpu.VMEM((2, TB, P), bf16),
            pltpu.VMEM((8, TB, 128), f32),
            pltpu.VMEM((4, TB, 128), f32),
            pltpu.VMEM((NB, TB, D), ODT),
            pltpu.SemaphoreType.DMA((7 + NB,)),
            pltpu.SemaphoreType.DMA((1,)),
        ],
        compiler_params=pltpu.CompilerParams(
            vmem_limit_bytes=100 * 1024 * 1024,
        ),
    )(x, A_Lambda_re, A_Lambda_im, A_B_re, A_B_im, A_C_re, A_C_im,
      A_log_dt, A_Dskip, B_w_gate.T, B_w_up.T, B_w_down, gate_w)
    return out.reshape(1, T, D)
```

```python
import numpy as np
import jax
import jax.numpy as jnp
from jax import lax
import jax.experimental.pallas as pl
import jax.experimental.pallas.tpu as pltpu

T, D, P, F = 2048, 512, 512, 1376
TB = 512
NB = T // TB
LC = TB // 8
FC = 256
FA = 1280
FR = F - FA
FCH = [(c0, c0 + FC) for c0 in range(0, FA, FC)]
OSPLIT = 4
NT = (((1,), (1,)), ((), ()))
f32 = jnp.float32
bf16 = jnp.bfloat16
C1 = float(np.sqrt(2.0 / np.pi))
C2 = float(np.sqrt(2.0 / np.pi) * 0.044715)

WGROUPS = ["x0,r", "b0", "b1", "b2", "b3", "f0", "f1", "f2", "f3", "c", "f4", "d"]
ORDER0 = ("R Z2 W1 B0 W2 B1 W3 B2 W4 B3 S0 S1 S2 S3 W5 F0 W6 F1 W7 F2 W8 F3 G W9 P W10 F4 "
          "C0 C1 C2 C3 W11 D0 D1 O0 D2 O1 D3 O2 O3").split()
ORDERN = ("B0 S0 F0 B1 S1 F1 B2 S2 F2 B3 S3 F3 F4 G C0 R C1 C2 C3 "
          "D0 D1 O0 D2 O1 D3 O2 O3").split()

_NEW_TOOLCHAIN = tuple(int(v) for v in jax.__version__.split(".")[:2]) >= (0, 12)
_FLAG_KW = {"flags": {"XLA_TPU_RESCHEDULE_DMA_DONES": True}} if _NEW_TOOLCHAIN else {}


def _cmac(ar, ai, hr, hi, ur, ui):
    return ur + (ar * hr - ai * hi), ui + (ar * hi + ai * hr)


def _kernel(x_h, lre_h, lim_h, bre_h, bim_h, cre_h, cim_h, ldt_h, dsk_h, wg_h, wu_h, wd_h, gw_h, o_h,
            x_s, vec_s, b_s, c_s, ct_s, wg_s, wu_s, wr_s, wd_s, act_s, tab_s, h_s, hb_s, us, ys, out_s,
            sems, osem):
    mk = pltpu.make_async_copy

    cp_vec = [mk(h, vec_s[n], sems.at[0]) for n, h in enumerate((lre_h, lim_h, ldt_h, dsk_h, gw_h))]
    grp = dict(x0=[(x_h.at[0:TB], x_s.at[0])])
    for q in range(4):
        grp["b%d" % q] = [((bre_h, bim_h)[k].at[128 * q:128 * q + 128], b_s.at[k, 128 * q:128 * q + 128])
                          for k in range(2)]
    for n, (c0, c1) in enumerate(FCH):
        grp["f%d" % n] = [(h.at[c0:c1], s.at[c0:c1]) for h, s in ((wg_h, wg_s), (wu_h, wu_s))]
    grp["r"] = [(h.at[FA:F], wr_s.at[n * FR:(n + 1) * FR]) for n, h in enumerate((wg_h, wu_h))]
    grp["c"] = [((cre_h, cim_h)[k], c_s.at[k]) for k in range(2)]
    grp["d"] = [(wd_h, wd_s)]
    waits = [[mk(src, dst, sems.at[1 + wi]) for g in w.split(",") for (src, dst) in grp[g]]
             for wi, w in enumerate(WGROUPS)]
    for cps in [cp_vec] + waits:
        for c in cps:
            c.start()
    ns = 1 + len(WGROUPS)
    for b in range(1, NB):
        mk(x_h.at[b * TB:(b + 1) * TB], x_s.at[b], sems.at[ns + b]).start()

    for c in cp_vec:
        c.wait()
    lre = vec_s[0][...].reshape(1, P).astype(f32)
    lim = vec_s[1][...].reshape(1, P).astype(f32)
    dt = jnp.exp(vec_s[2][...].reshape(1, P).astype(f32)).astype(bf16).astype(f32)
    zr = dt * lre
    zi = dt * lim
    mag = jnp.exp(zr)
    ar = mag * jnp.cos(zi)
    ai = mag * jnp.sin(zi)
    sub8 = lax.broadcasted_iota(jnp.int32, (8, P), 0)
    sf = ((sub8 + 1) * LC).astype(f32)
    mg = jnp.exp(sf * zr)
    pr = mg * jnp.cos(sf * zi)
    pi = mg * jnp.sin(sf * zi)
    den = 1.0 / (lre * lre + lim * lim)
    nr = ar - 1.0
    cr2 = 2.0 * (nr * lre + ai * lim) * den
    ci2 = 2.0 * (ai * lre - nr * lim) * den
    tab_s[0] = pr
    tab_s[1] = pi
    for n, k in enumerate((1, 2, 4)):
        kr = jnp.broadcast_to(pr[k - 1:k, :], (8, P))
        ki = jnp.broadcast_to(pi[k - 1:k, :], (8, P))
        tab_s[2 + 2 * n] = jnp.where(sub8 >= k, kr, 0.0)
        tab_s[3 + 2 * n] = jnp.where(sub8 >= k, ki, 0.0)
    tab_s[8] = jnp.broadcast_to(ar, (8, P))
    tab_s[9] = jnp.broadcast_to(ai, (8, P))
    tab_s[10] = jnp.broadcast_to(cr2, (8, P))
    tab_s[11] = jnp.broadcast_to(ci2, (8, P))
    h_s[...] = jnp.zeros(h_s.shape, f32)

    def body(b, first):
        if first:
            for c in waits[0]:
                c.wait()
        x = x_s[b]
        st = {}

        def perm_rows(m):
            c, jb = divmod(m, LC // 8)
            return pl.ds(64 * jb + c, 8, stride=8)

        def bproj(q):
            sl = slice(128 * q, 128 * q + 128)
            for k in range(2):
                u = lax.dot_general(x, b_s[k, sl, :], NT, preferred_element_type=f32)
                for m in range(TB // 8):
                    us[2 * q + k, perm_rows(m), :] = u[8 * m:8 * m + 8, :]

        def scan(q):
            sl = slice(128 * q, 128 * q + 128)
            lr = tab_s[8, :, sl]
            li = tab_s[9, :, sl]

            def u_at(j):
                return us[2 * q, 8 * j:8 * j + 8, :], us[2 * q + 1, 8 * j:8 * j + 8, :]

            er, ei = u_at(0)
            for j in range(1, LC):
                er, ei = _cmac(lr, li, er, ei, *u_at(j))
            for n, k in enumerate((1, 2, 4)):
                er, ei = _cmac(tab_s[2 + 2 * n, :, sl], tab_s[3 + 2 * n, :, sl],
                               pltpu.roll(er, k, 0), pltpu.roll(ei, k, 0), er, ei)
            h0r = h_s[0, :, sl]
            h0i = h_s[1, :, sl]
            er, ei = _cmac(tab_s[0, :, sl], tab_s[1, :, sl], h0r, h0i, er, ei)
            h_s[0, :, sl] = jnp.broadcast_to(er[7:8, :], (8, 128))
            h_s[1, :, sl] = jnp.broadcast_to(ei[7:8, :], (8, 128))
            sub = lax.broadcasted_iota(jnp.int32, (8, 128), 0)
            hr = jnp.where(sub == 0, h0r, pltpu.roll(er, 1, 0))
            hi = jnp.where(sub == 0, h0i, pltpu.roll(ei, 1, 0))
            for j in range(0, LC, 2):
                r0, i0 = _cmac(lr, li, hr, hi, *u_at(j))
                hr, hi = _cmac(lr, li, r0, i0, *u_at(j + 1))
                hb_s[0, 8 * j:8 * j + 16, sl] = jnp.concatenate([r0, hr], axis=0).astype(bf16)
                hb_s[1, 8 * j:8 * j + 16, sl] = jnp.concatenate([i0, hi], axis=0).astype(bf16)

        def geglu2(g, u):
            z = g * (C1 + C2 * (g * g))
            gu = g * u
            return gu + gu * jnp.tanh(z)

        def ffn(n):
            c0, c1 = FCH[n]
            g = lax.dot_general(x, wg_s[c0:c1, :], NT, preferred_element_type=f32)
            u = lax.dot_general(x, wu_s[c0:c1, :], NT, preferred_element_type=f32)
            act_s[:, c0:c1] = geglu2(g, u).astype(bf16)

        def ffn_rem():
            gu = lax.dot_general(wr_s[...], x, NT, preferred_element_type=f32)
            st["rgu"] = gu
            act_s[:, FA:F] = geglu2(gu[0:FR], gu[FR:2 * FR]).T.astype(bf16)

        def cprep():
            c_r = tab_s[10, 0:1, :]
            c_i = tab_s[11, 0:1, :]
            cre = c_s[0].astype(f32)
            cim = c_s[1].astype(f32)
            ct_s[0] = (cre * c_r - cim * c_i).astype(bf16)
            ct_s[1] = (-(cre * c_i + cim * c_r)).astype(bf16)

        def gate():
            xf = x.astype(f32)
            gl = jnp.sum(xf * vec_s[4][...].reshape(1, D).astype(f32), axis=-1, keepdims=True)
            st["xf"] = xf
            st["g"] = jax.nn.sigmoid(gl)
            st["dsk"] = vec_s[3][...].reshape(1, D).astype(f32)

        def cproj(n):
            sl = slice(128 * n, 128 * n + 128)
            y = lax.dot_general(hb_s[0], ct_s[0, sl, :], NT, preferred_element_type=f32)
            ys[n] = y + lax.dot_general(hb_s[1], ct_s[1, sl, :], NT, preferred_element_type=f32)

        def dproj(n):
            sl = slice(128 * n, 128 * n + 128)
            st["acc", n] = jnp.dot(act_s[...], wd_s[:, sl], preferred_element_type=f32)

        def mix(n):
            sl = slice(128 * n, 128 * n + 128)
            g = st["g"]
            rp = TB // (OSPLIT if n == 3 else 1)
            for r0 in range(0, TB, rp):
                rows = slice(r0, r0 + rp)
                y = jnp.concatenate([ys[n, perm_rows(m), :] for m in range(r0 // 8, (r0 + rp) // 8)], axis=0)
                y = y + st["xf"][rows, sl] * st["dsk"][:, sl]
                out_s[b, rows, sl] = g[rows] * y + (0.5 - 0.5 * g[rows]) * st["acc", n][rows]
                mk(out_s.at[b, rows, sl], o_h.at[pl.ds(b * TB + r0, rp), sl], osem.at[0]).start()

        for tok in (ORDER0 if first else ORDERN):
            k, n = tok[0], int(tok[1:] or 0)
            if k == "W":
                for c in waits[n]:
                    c.wait()
            elif k == "Z":
                b_s[0, P:P + 16, 0:128] = st["rgu"][0:16, 128 * n:128 * n + 128].astype(bf16)
            elif k == "B":
                bproj(n)
            elif k == "S":
                scan(n)
            elif k == "F":
                ffn(n)
            elif k == "R":
                ffn_rem()
            elif k == "P":
                cprep()
            elif k == "G":
                gate()
            elif k == "C":
                cproj(n)
            elif k == "D":
                dproj(n)
            elif k == "O":
                mix(n)

    body(0, True)

    def loop(b, carry):
        mk(x_h.at[pl.ds(b * TB, TB)], x_s.at[b], sems.at[ns + b]).wait()
        body(b, False)
        return carry

    lax.fori_loop(1, NB, loop, 0)
    mk(out_s, out_s, osem.at[0]).wait()


@jax.jit
def pallas_gated_mix__ssm_conv_s5__geglu_ffn__prompt_kernel(
    A_x, A_Lambda_re, A_Lambda_im, A_B_re, A_B_im, A_C_re, A_C_im, A_log_dt, A_Dskip,
    B_x, B_w_gate, B_w_up, B_w_down, gate_w,
):
    del B_x
    hbm = pl.BlockSpec(memory_space=pltpu.HBM)
    out = pl.pallas_call(
        _kernel,
        in_specs=[hbm] * 13,
        out_specs=hbm,
        out_shape=jax.ShapeDtypeStruct((T, D), f32),
        scratch_shapes=[
            pltpu.VMEM((NB, TB, D), bf16),
            [pltpu.VMEM((512,), bf16)] * 5,
            pltpu.VMEM((2, P + 16, D), bf16),
            pltpu.VMEM((2, D, P), bf16),
            pltpu.VMEM((2, D, P), bf16),
            pltpu.VMEM((FA, D), bf16),
            pltpu.VMEM((FA, D), bf16),
            pltpu.VMEM((2 * FR, D), bf16),
            pltpu.VMEM((F, D), bf16),
            pltpu.VMEM((TB, F), bf16),
            pltpu.VMEM((12, 8, P), f32),
            pltpu.VMEM((2, 8, P), f32),
            pltpu.VMEM((2, TB, P), bf16),
            pltpu.VMEM((8, TB, 128), f32),
            pltpu.VMEM((4, TB, 128), f32),
            pltpu.VMEM((NB, TB, D), f32),
            pltpu.SemaphoreType.DMA((1 + len(WGROUPS) + NB,)),
            pltpu.SemaphoreType.DMA((1,)),
        ],
        compiler_params=pltpu.CompilerParams(
            vmem_limit_bytes=100 * 1024 * 1024,
            **_FLAG_KW,
        ),
    )(A_x.reshape(T, D), A_Lambda_re, A_Lambda_im, A_B_re, A_B_im, A_C_re, A_C_im,
      A_log_dt, A_Dskip, B_w_gate.T, B_w_up.T, B_w_down, gate_w)
    return out.reshape(1, T, D)
```
